```python
import os as _os
_os.environ.setdefault("JAX_PLATFORMS", "cpu")
import jax
import jax.numpy as jnp

def _softmax(x, axis=-1):
    return jax.nn.softmax(x, axis=axis)
def _gelu(x):
    return jax.nn.gelu(x, approximate=True)
def _silu(x):
    return jax.nn.silu(x)
def _sigmoid(x):
    return jax.nn.sigmoid(x)
def _layernorm(x, axis=-1, eps=1e-5):
    m = jnp.mean(x, axis=axis, keepdims=True)
    v = jnp.var(x, axis=axis, keepdims=True)
    return (x - m) / jnp.sqrt(v + eps)
def _scatter_add(tgt, idx, src, axis=0):
    return tgt.at[idx].add(src)
def _segment_sum(src, seg, n):
    return jax.ops.segment_sum(src, seg, n)
class _Rng:
    def __init__(self, key):
        self._k = key
    def _next(self):
        self._k, sub = jax.random.split(self._k)
        return sub
    def normal(self, shape):
        return jax.random.normal(self._next(), shape, dtype=jnp.bfloat16)
    def randint(self, lo, hi, shape):
        return jax.random.randint(self._next(), shape, lo, hi, dtype=jnp.int32)
    def uniform(self, shape, lo=0.0, hi=1.0):
        return jax.random.uniform(self._next(), shape, jnp.bfloat16, lo, hi)
    def permutation(self, n):
        return jax.random.permutation(self._next(), n)


kernel_name = 'sequential_preLN__linear_attn_block__glu_gated_reglu__prompt'

def setup_inputs():
    _rng = _Rng(jax.random.key(int.from_bytes(__import__("os").urandom(4), "little")))
    _w = (lambda a: (lambda t: t.astype(jnp.bfloat16) if jnp.issubdtype(t.dtype, jnp.floating) else t)(jnp.asarray(a)))
    def _A_setup():
        B, S, D = 1, 2048, 640
        return {
            "x": _w((lambda *s: _rng.normal(s) * 0.05)(B, S, D)),
            "wqkv": _w((lambda *s: _rng.normal(s) * 0.05)(D, 3 * D)),
            "wo": _w((lambda *s: _rng.normal(s) * 0.05)(D, D)),
        }
    _A_in = _A_setup()

    def _B_setup():
        B, S, D, F = 1, 2048, 640, 1536
        return {
            "x": _w((lambda *s: _rng.normal(s) * 0.05)(B, S, D)),
            "W_gate": _w((lambda *s: _rng.normal(s) * 0.05)(D, F) * (2.0 / D) ** 0.5),
            "W_up": _w((lambda *s: _rng.normal(s) * 0.05)(D, F) * (2.0 / D) ** 0.5),
            "W_down": _w((lambda *s: _rng.normal(s) * 0.05)(F, D) * (1.0 / F) ** 0.5),
        }
    _B_in = _B_setup()

    return {
        "A_x": _A_in["x"],
        "A_wqkv": _A_in["wqkv"],
        "A_wo": _A_in["wo"],
        "B_x": _B_in["x"],
        "B_W_gate": _B_in["W_gate"],
        "B_W_up": _B_in["W_up"],
        "B_W_down": _B_in["W_down"],
    }

def reference(A_x, A_wqkv, A_wo, B_x, B_W_gate, B_W_up, B_W_down):
    def _A_ref(x, wqkv, wo):
        B, S, D = x.shape
        H = 32; Dh = D // H
        qkv = (lambda x, *d: x.transpose(*d))((x @ wqkv).reshape(B, S, 3, H, Dh), 2, 0, 3, 1, 4)
        q, k, v = qkv[0], qkv[1], qkv[2]
        phi = lambda t: jnp.where(t > 0, t + 1, jnp.exp(t)) + 1e-6
        pq, pk = phi(q), phi(k)
        kv = jnp.einsum("bhsd,bhse->bhde", pk, v)
        z = jnp.einsum("bhsd->bhd", pk)
        num = jnp.einsum("bhqd,bhde->bhqe", pq, kv)
        den = jnp.einsum("bhqd,bhd->bhq", pq, z)[..., None] + 1e-6
        o = num / den
        return (lambda x, *d: x.transpose(*d))(o, 0, 2, 1, 3).reshape(B, S, D) @ wo

    def _B_ref(x, W_gate, W_up, W_down):
        gate = jnp.einsum("bsd,df->bsf", x, W_gate)
        up = jnp.einsum("bsd,df->bsf", x, W_up)
        gate = gate * (lambda x, dt: x.astype(dt))(gate > 0, gate.dtype)
        h = gate * up
        return jnp.einsum("bsf,fd->bsd", h, W_down)

    x = A_x
    h = x + _A_ref(_layernorm(x, axis=-1), A_wqkv, A_wo)
    h2 = h + _B_ref(_layernorm(h, axis=-1), B_W_gate, B_W_up, B_W_down)
    return h2
```

```python
import jax
import jax.numpy as jnp
from jax import lax
import jax.experimental.pallas as pl
import jax.experimental.pallas.tpu as pltpu

S, D, F, H, DH = 2048, 640, 1536, 32, 20
T1 = 512
T2 = 512
TP = 128
PC1 = [(0,128),(128,384)]
PC2 = [(0, 256), (256, 256)]
NP = T2 // TP
BF, F32 = jnp.bfloat16, jnp.float32


def _ranges():
    out = []
    for j in range(D // 128):
        lo = (128 * j // DH) * DH
        hi = -(-(128 * (j + 1)) // DH) * DH
        lo = lo // 16 * 16
        hi = min(-(-hi // 16) * 16, D)
        out.append((lo, hi))
    return out


RANGES = _ranges()


def _ln(x):
    m = jnp.mean(x, axis=-1, keepdims=True)
    xc = x - m
    v = jnp.mean(xc * xc, axis=-1, keepdims=True)
    return xc * lax.rsqrt(v + 1e-5)


def _phi(t):
    return jnp.where(t > 0, t + 1.0, jnp.exp(t)) + 1e-6


def _head(i):
    return (i * 3277) >> 16


def _dot(a, b):
    return jnp.dot(a, b, preferred_element_type=F32)


def _body(x_hbm, wqkv_hbm, wo_hbm, wg_hbm, wu_hbm, wd_hbm, out_hbm,
          x_vm, wq_vm, wk_vm, wv_vm, wkT_vm, wo_vm, wg_vm, wu_vm, wd_vm,
          pq_vm, out_vm, g_vm, z_vm, m_vm, zb_vm, e_vm, xsem, wsem, osem):
    n1, n2 = S // T1, S // T2

    def x_copy(i):
        return pltpu.make_async_copy(x_hbm.at[pl.ds(i * T1, T1), :], x_vm.at[pl.ds(i * T1, T1), :], xsem.at[i])

    cq = pltpu.make_async_copy(wqkv_hbm.at[:, pl.ds(0, D)], wq_vm, wsem.at[0])
    ck = pltpu.make_async_copy(wqkv_hbm.at[:, pl.ds(D, D)], wk_vm, wsem.at[1])
    cv = pltpu.make_async_copy(wqkv_hbm.at[:, pl.ds(2 * D, D)], wv_vm, wsem.at[2])
    co = pltpu.make_async_copy(wo_hbm, wo_vm, wsem.at[3])
    cg = pltpu.make_async_copy(wg_hbm, wg_vm, wsem.at[4])
    cu = pltpu.make_async_copy(wu_hbm, wu_vm, wsem.at[5])
    cd = pltpu.make_async_copy(wd_hbm, wd_vm, wsem.at[6])

    x_copy(0).start()
    cq.start()

    def p1h(rows, first):
        lnx = _ln(x_vm[rows, :].astype(F32)).astype(BF)
        if first:
            cq.wait()
        pq_vm[rows, :] = _phi(_dot(lnx, wq_vm[...])).astype(BF)
        if first:
            ck.wait()
            for t in range(1, n1):
                x_copy(t).start()
            wkT_vm[...] = wk_vm[...].T
        kT = lax.dot_general(wkT_vm[...], lnx, (((1,), (1,)), ((), ())), preferred_element_type=F32)
        if first:
            cv.start()
            co.start()
            cg.start()
            cu.start()
            cd.start()
        return _phi(kT), lnx

    def kvacc(pkT, lnx, first):
        zs = pkT[:, 0:128]
        for c0 in range(128, pkT.shape[1], 128):
            zs = zs + pkT[:, c0:c0 + 128]
        g = _dot(pkT.astype(BF), lnx)
        if first:
            z_vm[...] = zs
            g_vm[...] = g
        else:
            z_vm[...] += zs
            g_vm[...] += g

    def p1(i, first):
        x_copy(i).wait()
        if first:
            ck.start()
            kvacc(*p1h(pl.ds(0, T1), True), True)
        else:
            r = [p1h(pl.ds(pl.multiple_of(i * T1 + o, 128), n), False) for o, n in PC1]
            kvacc(jnp.concatenate([t[0] for t in r], axis=1), jnp.concatenate([t[1] for t in r], axis=0), False)

    p1(0, True)
    lax.fori_loop(1, n1, lambda i, c: (p1(i, False), c)[1], 0)

    cv.wait()
    co.wait()
    m_vm[...] = jnp.zeros(m_vm.shape, F32)
    for j, (lo, hi) in enumerate(RANGES):
        r = lax.broadcasted_iota(jnp.int32, (hi - lo, 128), 0) + lo
        c = lax.broadcasted_iota(jnp.int32, (hi - lo, 128), 1) + 128 * j
        kv = _dot(g_vm[lo:hi, :].astype(BF), wv_vm[:, 128 * j:128 * (j + 1)])
        kvj = jnp.where(_head(r) == _head(c), kv, 0.0).astype(BF)
        m_vm[lo:hi, :] += _dot(kvj, wo_vm[128 * j:128 * (j + 1), :])
    wo_vm[...] = m_vm[...].astype(BF)
    z = jnp.sum(z_vm[...], axis=-1, keepdims=True)
    r = lax.broadcasted_iota(jnp.int32, (D, 128), 0)
    c = lax.broadcasted_iota(jnp.int32, (D, 128), 1)
    zb_vm[...] = jnp.where(_head(r) == c, jnp.broadcast_to(z, (D, 128)), 0.0).astype(BF)
    r = lax.broadcasted_iota(jnp.int32, (128, D), 0)
    c = lax.broadcasted_iota(jnp.int32, (128, D), 1)
    e_vm[...] = jnp.where(r == _head(c), 1.0, 0.0).astype(BF)

    cg.wait()
    cu.wait()
    cd.wait()

    def attn(rows):
        pq = pq_vm[rows, :]
        den = _dot(pq, zb_vm[...])
        rc = (1.0 / (den + 1e-6)).astype(BF)
        on = (pq.astype(F32) * _dot(rc, e_vm[...])).astype(BF)
        h = x_vm[rows, :].astype(F32) + _dot(on, wo_vm[...])
        return h, _ln(h).astype(BF)

    def ffn(h, lnh):
        g = _dot(lnh, wg_vm[...])
        u = _dot(lnh, wu_vm[...])
        a = (jnp.maximum(g, 0.0) * u).astype(BF)
        return (h + _dot(a, wd_vm[...])).astype(BF)

    def emit(i, o, p0, npc):
        for p in range(npc):
            r = pl.ds(pl.multiple_of(i * T2 + (p0 + p) * TP, TP), TP)
            out_vm[r, :] = o[p * TP:(p + 1) * TP, :]
            pltpu.make_async_copy(out_vm.at[r, :], out_hbm.at[r, :], osem.at[i * NP + p0 + p]).start()

    def p2(i, c):
        hl = [attn(pl.ds(pl.multiple_of(i * T2 + o, 128), n)) for o, n in PC2]
        p0 = 0
        for h, l in hl:
            emit(i, ffn(h, l), p0, h.shape[0] // TP)
            p0 += h.shape[0] // TP
        return c

    lax.fori_loop(0, n2, p2, 0)
    for i in range(n2 * NP):
        pltpu.make_async_copy(out_vm.at[pl.ds(i * TP, TP), :], out_hbm.at[pl.ds(i * TP, TP), :], osem.at[i]).wait()


@jax.jit
def pallas_sequential_preLN__linear_attn_block__glu_gated_reglu__prompt_kernel(
    A_x, A_wqkv, A_wo, B_x, B_W_gate, B_W_up, B_W_down,
):
    x2 = A_x.reshape(S, D)
    any_spec = pl.BlockSpec(memory_space=pl.ANY)
    out = pl.pallas_call(
        _body,
        in_specs=[any_spec] * 6,
        out_specs=any_spec,
        out_shape=jax.ShapeDtypeStruct((S, D), BF),
        scratch_shapes=[
            pltpu.VMEM((S, D), BF),
            pltpu.VMEM((D, D), BF),
            pltpu.VMEM((D, D), BF),
            pltpu.VMEM((D, D), BF),
            pltpu.VMEM((D, D), BF),
            pltpu.VMEM((D, D), BF),
            pltpu.VMEM((D, F), BF),
            pltpu.VMEM((D, F), BF),
            pltpu.VMEM((F, D), BF),
            pltpu.VMEM((S, D), BF),
            pltpu.VMEM((S, D), BF),
            pltpu.VMEM((D, D), F32),
            pltpu.VMEM((D, 128), F32),
            pltpu.VMEM((D, D), F32),
            pltpu.VMEM((D, 128), BF),
            pltpu.VMEM((128, D), BF),
            pltpu.SemaphoreType.DMA((S // T1,)),
            pltpu.SemaphoreType.DMA((7,)),
            pltpu.SemaphoreType.DMA((S // TP,)),
        ],
        compiler_params=pltpu.CompilerParams(vmem_limit_bytes=100 * 1024 * 1024),
    )(x2, A_wqkv, A_wo, B_W_gate, B_W_up, B_W_down)
    return out.reshape(1, S, D)
```
